```python
import jax
import jax.numpy as jnp

def _softmax(x, axis=-1):
    return jax.nn.softmax(x, axis=axis)
def _gelu(x):
    return jax.nn.gelu(x, approximate=True)
def _silu(x):
    return jax.nn.silu(x)
def _sigmoid(x):
    return jax.nn.sigmoid(x)
def _layernorm(x, axis=-1, eps=1e-5):
    m = jnp.mean(x, axis=axis, keepdims=True)
    v = jnp.var(x, axis=axis, keepdims=True)
    return (x - m) / jnp.sqrt(v + eps)
def _scatter_add(tgt, idx, src, axis=0):
    return tgt.at[idx].add(src)
def _segment_sum(src, seg, n):
    return jax.ops.segment_sum(src, seg, n)
class _Rng:
    def __init__(self, key):
        self._k = key
    def _next(self):
        self._k, sub = jax.random.split(self._k)
        return sub
    def normal(self, shape):
        return jax.random.normal(self._next(), shape, dtype=jnp.bfloat16)
    def randint(self, lo, hi, shape):
        return jax.random.randint(self._next(), shape, lo, hi, dtype=jnp.int32)
    def uniform(self, shape, lo=0.0, hi=1.0):
        return jax.random.uniform(self._next(), shape, jnp.bfloat16, lo, hi)
    def permutation(self, n):
        return jax.random.permutation(self._next(), n)


kernel_name = 'sequential_preLN__sliding_block__glu_gated_glu__prompt'

def _fwd_setup_inputs():
    _rng = _Rng(jax.random.key(int.from_bytes(__import__("os").urandom(4), "little")))
    _w = (lambda a: (lambda t: t.astype(jnp.bfloat16) if jnp.issubdtype(t.dtype, jnp.floating) else t)(jnp.asarray(a)))
    def _A_setup():
        B, S, D = 1, 2048, 512
        return {
            "x": _w((lambda *s: _rng.normal(s) * 0.05)(B, S, D)),
            "wqkv": _w((lambda *s: _rng.normal(s) * 0.05)(D, 3 * D)),
            "wo": _w((lambda *s: _rng.normal(s) * 0.05)(D, D)),
        }
    _A_in = _A_setup()

    def _B_setup():
        B, S, D, F = 1, 2048, 512, 1376
        return {
            "x": _w((lambda *s: _rng.normal(s) * 0.05)(B, S, D)),
            "w_gate": _w((lambda *s: _rng.normal(s) * 0.05)(D, F)),
            "w_up": _w((lambda *s: _rng.normal(s) * 0.05)(D, F)),
            "w_down": _w((lambda *s: _rng.normal(s) * 0.05)(F, D)),
        }
    _B_in = _B_setup()

    return {
        "A_x": _A_in["x"],
        "A_wqkv": _A_in["wqkv"],
        "A_wo": _A_in["wo"],
        "B_x": _B_in["x"],
        "B_w_gate": _B_in["w_gate"],
        "B_w_up": _B_in["w_up"],
        "B_w_down": _B_in["w_down"],
    }

def _fwd_reference(A_x, A_wqkv, A_wo, B_x, B_w_gate, B_w_up, B_w_down):
    def _A_ref(x, wqkv, wo):
        B, S, D = x.shape
        H = 32; Dh = D // H; W = 256
        qkv = (lambda x, *d: x.transpose(*d))((x @ wqkv).reshape(B, S, 3, H, Dh), 2, 0, 3, 1, 4)
        q, k, v = qkv[0], qkv[1], qkv[2]
        scores = jnp.einsum("bhqd,bhkd->bhqk", q, k) * (Dh ** -0.5)
        idx = jnp.arange(S)
        mask = (idx[:, None] - idx[None, :] >= 0) & (idx[:, None] - idx[None, :] < W)
        scores = jnp.where(mask[None, None], scores, -1e9)
        p = _softmax(scores, axis=-1)
        o = jnp.einsum("bhqk,bhkd->bhqd", p, v)
        return (lambda x, *d: x.transpose(*d))(o, 0, 2, 1, 3).reshape(B, S, D) @ wo

    def _B_ref(x, w_gate, w_up, w_down):
        g = jnp.einsum("bsd,df->bsf", x, w_gate)
        u = jnp.einsum("bsd,df->bsf", x, w_up)
        h = _sigmoid(g) * u
        return jnp.einsum("bsf,fd->bsd", h, w_down)

    x = A_x
    h = x + _A_ref(_layernorm(x, axis=-1), A_wqkv, A_wo)
    h2 = h + _B_ref(_layernorm(h, axis=-1), B_w_gate, B_w_up, B_w_down)
    return h2


def setup_inputs():
    _inp = _fwd_setup_inputs()
    _gk = jax.random.fold_in(jax.random.key(int.from_bytes(__import__("os").urandom(4), "little")), 2**31 - 1)
    _shapes = [[1, 2048, 512]]
    _dtypes = ['bfloat16']
    _gks = jax.random.split(_gk, len(_shapes))
    _gs = [jax.random.normal(k, s, dtype=jnp.dtype(d)) * 0.05 for k, s, d in zip(_gks, _shapes, _dtypes)]
    _inp["grad_out"] = _gs[0]
    return _inp

def reference(A_x, A_wqkv, A_wo, B_w_gate, B_w_up, B_w_down, B_x, grad_out):
    _const = dict(B_x=B_x)
    def _f(*_d):
        return _fwd_reference(**{'A_x': _d[0], 'A_wqkv': _d[1], 'A_wo': _d[2], 'B_w_gate': _d[3], 'B_w_up': _d[4], 'B_w_down': _d[5], **_const})
    _out, _vjp = jax.vjp(_f, A_x, A_wqkv, A_wo, B_w_gate, B_w_up, B_w_down)
    _grads = _vjp(grad_out)
    _out0 = jnp.asarray(_out)
    return (_out0, *[jnp.asarray(_g) for _g in _grads])
```

```python
import jax
import jax.numpy as jnp
from jax import lax
import jax.experimental.pallas as pl
import jax.experimental.pallas.tpu as pltpu

S, D, F = 2048, 512, 1376
W = 256
TB = 256
NB = S // TB
NSUB = TB // 128
FP = 1408
FC = 256
EPS = 1e-5
LOG2E = 1.4426950408889634
QSCALE = 0.25 * LOG2E
BF, F32 = jnp.bfloat16, jnp.float32
NN = (((1,), (0,)), ((), ()))
NT = (((1,), (1,)), ((), ()))


def _nn(a, b):
    return lax.dot_general(a, b, NN, preferred_element_type=F32)


def _nt(a, b):
    return lax.dot_general(a, b, NT, preferred_element_type=F32)


def _ln(x):
    m = jnp.mean(x, axis=-1, keepdims=True)
    xc = x - m
    rstd = lax.rsqrt(jnp.mean(xc * xc, axis=-1, keepdims=True) + EPS)
    return xc * rstd, rstd


def _ln_bwd(dy, xh, rstd):
    m1 = jnp.mean(dy, axis=-1, keepdims=True)
    m2 = jnp.mean(dy * xh, axis=-1, keepdims=True)
    return rstd * (dy - m1 - xh * m2)


def _ds(start, size, mult):
    return pl.ds(pl.multiple_of(start, mult), size)


def _kernel(x_h, wqkv_h, wo_h, wg_h, wu_h, wd_h, go_h,
            out_h, dx_h, dwqkv_h, dwo_h, dwg_h, dwu_h, dwd_h,
            x_v, go_v, wqo, w3,
            k_n, v_n, k_t, k_s, v_t, v_s, q_t, dq_t,
            dka, dkb, dva, dvb, p_v, linv,
            act3, lhs1, lhs2, do_t, dh_v,
            h_v, acc_o, acc_d, out_st, dqkv_t, s_scr, m_scr, ds_scr, tmp,
            isem, osem):
    wqkv, wo = wqo.at[:, 0:3 * D], wqo.at[:, 3 * D:4 * D]
    OG, OU, OD = 0, FP, 2 * FP
    wg, wu, wd = (w3.at[o:o + F] for o in (OG, OU, OD))
    ln1_t, o_t = lhs1.at[0], lhs1.at[1]
    ln2_t, go_t = lhs2.at[0], lhs2.at[1]
    now = pl.when(pl.program_id(0) == 0)

    in_copies = [
        pltpu.make_async_copy(x_h.at[0:TB], x_v.at[0:TB], isem.at[0]),
        pltpu.make_async_copy(wqkv_h.at[:, 0:D], wqo.at[:, 0:D], isem.at[1]),
        pltpu.make_async_copy(wo_h, wo, isem.at[2]),
        pltpu.make_async_copy(go_h.at[0:TB], go_v.at[0:TB], isem.at[3]),
        pltpu.make_async_copy(wg_h, wg, isem.at[4]),
        pltpu.make_async_copy(wu_h, wu, isem.at[5]),
        pltpu.make_async_copy(wd_h, wd, isem.at[6]),
        pltpu.make_async_copy(x_h.at[TB:2 * TB], x_v.at[TB:2 * TB], isem.at[7]),
        pltpu.make_async_copy(x_h.at[2 * TB:S], x_v.at[2 * TB:S], isem.at[8]),
        pltpu.make_async_copy(go_h.at[TB:S], go_v.at[TB:S], isem.at[9]),
        pltpu.make_async_copy(wqkv_h.at[:, D:2 * D], wqo.at[:, D:2 * D], isem.at[10]),
        pltpu.make_async_copy(wqkv_h.at[:, 2 * D:], wqo.at[:, 2 * D:3 * D], isem.at[11]),
    ]
    in_copies[0].start()
    in_copies[1].start()
    in_copies[10].start()
    in_copies[11].start()

    for r in (k_n, v_n):
        r[0:W // 2, :] = jnp.zeros((W // 2, D), jnp.int32)
    for r in (k_t, k_s, v_t, v_s):
        r[:, 0:W] = jnp.zeros((D, W), BF)

    def zero_acc(c0):
        for r in (*dka, *dkb, *dva, *dvb):
            r[:, _ds(c0, 256, 256)] = jnp.zeros((D // 4, 256), F32)
    zero_acc(0)
    for o in (OG, OU, OD):
        w3[o + F:o + FP, :] = jnp.zeros((FP - F, D), BF)

    row = lax.broadcasted_iota(jnp.int32, (64, 128), 0)
    lane = lax.broadcasted_iota(jnp.int32, (64, 128), 1)
    key = (row & 32) + 2 * (row & 15) + ((row >> 4) & 1)
    tri = key > (lane & 63)
    lo8 = lax.broadcasted_iota(jnp.int32, (8, 128), 1) < 64
    lo16 = lax.broadcasted_iota(jnp.int32, (16, 128), 1) < 64
    I32 = jnp.int32
    pk = lambda a, b: as_i(pltpu.pack_elementwise([a, b], packed_dtype=BF))
    upk = lambda w, j: pltpu.unpack_elementwise(w, index=j, packed_dtype=BF, unpacked_dtype=F32)
    as_i = lambda t: pltpu.bitcast(t, I32)
    as_b = lambda t: pltpu.bitcast(t, BF)

    def blockdiag(t, pair):
        h0 = t[pair * 16:pair * 16 + 8]
        h1 = t[pair * 16 + 8:pair * 16 + 16]
        ua = jnp.concatenate([jnp.where(lo8, h0, 0), jnp.where(lo8, 0, h1)], axis=0)
        ub = jnp.concatenate([jnp.where(lo8, 0, h0), jnp.where(lo8, h1, 0)], axis=0)
        return ua, ub

    def pad128(t, pair):
        parts = []
        if pair > 0:
            parts.append(jnp.zeros((16 * pair, 128), I32))
        parts.append(t)
        if pair < 3:
            parts.append(jnp.zeros((16 * (3 - pair), 128), I32))
        return as_b(jnp.concatenate(parts, axis=0))

    def skew_rows(ref, t0, hg, u):
        even = (lax.broadcasted_iota(I32, (160, 128), 1) & 16) == 0
        cols = _ds(hg * 128, 128, 128)
        r0 = ref[_ds(t0 // 2, 160, 64), cols]
        r1 = ref[_ds(t0 // 2 + 32, 160, 32), cols]
        return as_b(jnp.where(even, r0, r1) if u == 0 else jnp.where(even, r1, r0))

    def skew_t(ref_a, ref_s, t0, hg, pair):
        r0 = _ds(hg * 128 + pair * 32, 16, 16)
        r1 = _ds(hg * 128 + pair * 32 + 16, 16, 16)
        cols = _ds(t0, 256, 128)
        c1 = _ds(t0 + 128, 128, 128)
        c2 = _ds(t0 + 256, 128, 128)
        ua = jnp.concatenate([ref_a[r0, cols], ref_s[r1, cols]], axis=0)
        ub = jnp.concatenate([ref_s[r0, cols], ref_a[r1, cols]], axis=0)
        a0 = as_i(ref_a[r0, c2])
        tail = as_b(jnp.concatenate([
            jnp.where(lo8, a0, 0), jnp.where(lo8, as_i(ref_s[r1, c2]), 0),
            jnp.where(lo8, 0, a0), jnp.where(lo8, 0, as_i(ref_s[r1, c1]))], axis=0))
        return ua, ub, tail

    tr = lambda t: as_b(as_i(t.T) | pl.program_id(0))

    def keys_nn(lhs, pa, pb, pt):
        t = _nn(lhs[2], pt)
        return merge(_nn(lhs[0], pa) + t[:32], _nn(lhs[1], pb) + t[32:])

    def keys_nt(acc_a, acc_b, t0, hg, la, lb, pa, pb, pt):
        r0 = _ds(hg * 32, 16, 16)
        r1 = _ds(hg * 32 + 16, 16, 16)
        cols = _ds(t0, 256, 128)
        c2 = _ds(t0 + 256, 128, 128)
        ra, rb = _nn(la, tr(pa)), _nn(lb, tr(pb))
        t = _nn(jnp.concatenate([la, lb], axis=0), tr(pt))
        acc_a[r0, cols] += ra[:16]
        acc_a[r1, cols] += rb[16:]
        acc_b[r0, cols] += rb[:16]
        acc_b[r1, cols] += jnp.concatenate(
            [ra[16:, :128], ra[16:, 128:] + jnp.where(lo16, 0.0, t[48:])], axis=1)
        acc_a[r0, c2] += jnp.where(lo16, t[:16], t[32:48])
        acc_b[r1, c2] += jnp.where(lo16, t[16:32], 0.0)

    def merge(ra, rb):
        return jnp.concatenate([jnp.where(lo16, ra[:16], rb[:16]),
                                jnp.where(lo16, rb[16:], ra[16:])], axis=0)


    NIT = NSUB * 4

    def parts(ref, slot):
        return [as_b(ref[slot, a:a + n, :]) for a, n in ((0, 128), (128, 128), (256, 64))]

    def word0(u, r):
        return u * 128 + r // 2 if r < 256 else 256 + u * 32 + (r - 256) // 2

    def geo(i, it):
        sub = it // 4
        return sub, it % 4, i * TB + sub * 128

    def li_ref(it):
        return linv.at[_ds((it % 4) * 128, 128, 128), _ds((it // 4) * 128, 128, 128)]

    def scores(i, it, rmin):
        sub, hg, t0 = geo(i, it)
        q = as_i(q_t[_ds(hg * 128, 128, 128), _ds(t0, 128, 128)])
        for u in range(2):
            k = skew_rows(k_n, t0, hg, u)
            rhs = jnp.concatenate(
                [pad128(blockdiag(q, pp)[u], pp) for pp in range(4)], axis=1)
            if rmin:
                sa = _nn(k[rmin:320], rhs)
            else:
                sa = _nn(jnp.concatenate([k[o + r:o + r + 32] for r in (0, 32) for o in (0, 256)]
                                         + [k[64:256]], axis=0), rhs)
            sb = s_scr[u]
            for pp in range(4):
                ls = slice(pp * 128, (pp + 1) * 128)
                for r in (0, 32, *range(max(rmin, 64), 256, 32)):
                    if r >= 64:
                        o = r - rmin if rmin else r + 64
                        c = sa[o:o + 32, ls]
                        if rmin:
                            c = jnp.where(t0 + r + key[:32] + (lane[:32] & 64) >= W, c, -1e30)
                    elif rmin:
                        o = 256 + r - rmin
                        c = jnp.where(tri[r:r + 32], -1e30, sa[o:o + 32, ls])
                    else:
                        c = jnp.where(tri[r:r + 32], sa[2 * r:2 * r + 32, ls],
                                      sa[2 * r + 32:2 * r + 64, ls])
                    sb[r:r + 32, ls] = c
                    c = jnp.maximum(jnp.maximum(c[:8], c[8:16]), jnp.maximum(c[16:24], c[24:]))
                    m = c if r == 0 else jnp.maximum(m, c)
                m_scr[u][:, ls] = jnp.broadcast_to(
                    jnp.max(m, axis=0, keepdims=True), (8, 128))

    def softmax_pv(i, it, rmin):
        sub, hg, t0 = geo(i, it)
        slot = (i % 2) * NIT + it
        hist = []
        for pair in range(4):
            ls = slice(pair * 128, (pair + 1) * 128)
            li = []
            for u in range(2):
                sb = s_scr[u]
                m8 = m_scr[u][:, ls]
                for r in range(64, rmin, 32):
                    p_v[pair][slot, word0(u, r):word0(u, r) + 16, :] = jnp.zeros((16, 128), I32)
                for r in (0, 32, *range(max(rmin, 64), 256, 32)):
                    if len(hist) >= 3:
                        m8 = jnp.where(hist[-3] < 0.0, 0.0, m8)
                    m = jnp.concatenate([m8] * 4, axis=0)
                    e = jnp.exp2(sb[r:r + 32, ls] - m)
                    e8 = (e[:8] + e[8:16]) + (e[16:24] + e[24:])
                    l = e8 if r == 0 else l + e8
                    hist.append(l)
                    w0 = word0(u, r)
                    if r < 64:
                        e0 = jnp.where(tri[r:r + 32], e, 0.0)
                        e1 = jnp.where(tri[r:r + 32], 0.0, e)
                        w1 = word0(u, r + 256)
                        p_v[pair][slot, w0:w0 + 16, :] = pk(e0[:16], e0[16:])
                        p_v[pair][slot, w1:w1 + 16, :] = pk(e1[:16], e1[16:])
                    else:
                        p_v[pair][slot, w0:w0 + 16, :] = pk(e[:16], e[16:])
                li.append(jnp.broadcast_to(1.0 / jnp.sum(l, axis=0, keepdims=True), (8, 128)))
            h0, h1 = jnp.where(lo8, li[0], li[1]), jnp.where(lo8, li[1], li[0])
            li = jnp.concatenate([h0, h0, h1, h1], axis=0)
            li_ref(it)[pair * 32:pair * 32 + 32, :] = li
            r = keys_nn(skew_t(v_t, v_s, t0, hg, pair), *parts(p_v[pair], slot))
            o_t[_ds(hg * 128 + pair * 32, 32, 32), _ds(t0, 128, 128)] = (r * li).astype(BF)

    def dscores(i, it):
        sub, hg, t0 = geo(i, it)
        slot = (i % 2) * NIT + it
        rows, tg = _ds(hg * 128, 128, 128), _ds(t0, 128, 128)
        dof = do_t[rows, _ds(sub * 128, 128, 128)]
        prod = dof * o_t[rows, tg].astype(F32)
        do = as_i(dof.astype(BF))
        dos = [blockdiag(do, pp) for pp in range(4)]
        deltas = []
        for pair in range(4):
            d0 = jnp.sum(prod[pair * 32:pair * 32 + 16], axis=0, keepdims=True)
            d1 = jnp.sum(prod[pair * 32 + 16:pair * 32 + 32], axis=0, keepdims=True)
            deltas.append((jnp.where(lo8[0:1], d0, d1), jnp.where(lo8[0:1], d1, d0)))
        for u in range(2):
            dp = _nn(skew_rows(v_n, t0, hg, u), jnp.concatenate(
                [pad128(dos[pp][u], pp) for pp in range(4)], axis=1))
            for pair in range(4):
                delta = deltas[pair][u]
                for r in range(0, 320, 32):
                    w0 = word0(u, r)
                    w = p_v[pair][slot, w0:w0 + 16, :]
                    x = dp[r:r + 32, pair * 128:(pair + 1) * 128]
                    ds_scr[pair, w0:w0 + 16, :] = pk(
                        upk(w, 0) * (x[:16] - delta), upk(w, 1) * (x[16:] - delta))
        dvalues(i, it, dos)

    def dvalues(i, it, dos):
        sub, hg, t0 = geo(i, it)
        slot = (i % 2) * NIT + it
        for pair in range(4):
            keys_nt(dva[pair], dvb[pair], t0, hg, as_b(dos[pair][0]), as_b(dos[pair][1]),
                    *parts(p_v[pair], slot))

    def dqk(i, it):
        sub, hg, t0 = geo(i, it)
        rows, tg = _ds(hg * 128, 128, 128), _ds(t0, 128, 128)
        q = as_i(q_t[rows, tg])
        for pair in range(4):
            ds = parts(ds_scr, pair)
            dq_t[_ds(hg * 128 + pair * 32, 32, 32), tg] = keys_nn(
                skew_t(k_t, k_s, t0, hg, pair), *ds)
            qa, qb = blockdiag(q, pair)
            keys_nt(dka[pair], dkb[pair], t0, hg, as_b(qa), as_b(qb), *ds)

    def mlp_dw(j):
        c = _ds(j * 256, 256, 256)
        w3[c, :] = _nn(lhs2[j // 11], act3[:, c]).T.astype(BF)

    def attention(i, bwd, fwd):
        @pl.loop(0, NIT)
        def _(it):
            if bwd:
                dscores(i, it)
            if fwd:
                scores(i + 1, it, 0)
            if bwd:
                dqk(i, it)
            if fwd:
                softmax_pv(i + 1, it, 0)
            else:
                mlp_dw(it)

    out_copy = lambda i: pltpu.make_async_copy(
        out_st, out_h.at[_ds(i * TB, TB, TB), :], osem.at[0])

    def shifted(prev, cur):
        return jnp.concatenate([prev[:, 64:], cur[:, :TB - 64]], axis=1)

    def qkv(i):
        tok = _ds(i * TB, TB, TB)
        ptok = _ds(i * TB + W, TB, TB)
        xh, _ = _ln(x_v[tok, :].astype(F32))
        xb = xh.astype(BF)
        yield
        ln1_t[:, tok] = xh.T.astype(BF)
        q = _nn(xb, wqo[:, 0:D]) * QSCALE
        yield
        q_t[:, tok] = q.T.astype(BF)
        yield
        for j, (rn, rt, rs) in enumerate(((k_n, k_t, k_s), (v_n, v_t, v_s))):
            y = _nn(xb, wqo[:, (j + 1) * D:(j + 2) * D])
            for cb in range(4):
                tmp[cb] = y[:, cb * 128:(cb + 1) * 128]
            for cb in range(4):
                for r in range(0, TB, 64):
                    z = [tmp[cb, pl.ds(r + o, 16, stride=4), :] for o in range(4)]
                    wa, wb = pk(z[0], z[2]), pk(z[1], z[3])
                    rn[_ds((i * TB + W + r) // 2, 32, 32), cb * 128:(cb + 1) * 128] = (
                        jnp.concatenate([wa[:8], wb[:8], wa[8:], wb[8:]], axis=0))
            yt = y.T.astype(BF)
            rt[:, ptok] = yt
            rs[:, _ds(i * TB + W - 128, 128, 128)] = jnp.concatenate(
                [rs[:, _ds(i * TB + W - 128, 128, 128)][:, :64], yt[:, :64]], axis=1)
            rs[:, ptok] = jnp.concatenate([yt[:, 64:], jnp.zeros((D, 64), BF)], axis=1)
            yield


    in_copies[0].wait()

    first_qkv = qkv(0)
    next(first_qkv)
    in_copies[1].wait()
    next(first_qkv)
    next(first_qkv)
    in_copies[10].wait()
    next(first_qkv)
    in_copies[11].wait()

    @now
    def _():
        for cp in in_copies[2:8]:
            cp.start()
    next(first_qkv)
    for sub, rmin in enumerate((192, 64)):
        @pl.loop(4 * sub, 4 * sub + 4)
        def _(it):
            scores(it - it, it, rmin)
            softmax_pv(it - it, it, rmin)

    def block(i, c):
        tok = _ds(i * TB, TB, TB)
        ptok = _ds(i * TB + W, TB, TB)
        @pl.when(i == 0)
        def _():
            for cp in in_copies[2:8]:
                cp.wait()
            for cp in in_copies[8:10]:
                cp.start()

        @pl.when(i == 1)
        def _():
            for cp in in_copies[8:10]:
                cp.wait()

        @pl.when(i > 0)
        def _():
            out_copy(i - 1).wait()

        nxt = qkv(jnp.minimum(i + 1, NB - 1))
        for _ in range(1):
            next(nxt)
        h = x_v[tok, :].astype(F32) + _nn(o_t[:, tok].astype(F32).T.astype(BF), wqo[:, 3 * D:])
        for _ in range(2):
            next(nxt)
        hh, rstd2 = _ln(h)
        ln2_t[:, tok] = hh.T.astype(BF)
        hb = hh.astype(BF)
        gb = go_v[tok, :]
        acc_o[...] = h
        h_v[...] = hh
        for n, c0 in enumerate(range(0, FP, FC)):
            w = min(FC, FP - c0)
            cg, cu, cd = (slice(o + c0, o + c0 + w) for o in (OG, OU, OD))
            g = _nt(hb, w3[cg, :])
            uu = _nt(hb, w3[cu, :])
            da = _nt(gb, w3[cd, :])
            sg = 0.5 * jnp.tanh(0.5 * g) + 0.5
            a = sg * uu
            du = da * sg
            dg = a * (da - du)
            ab, dgb, dub = a.astype(BF), dg.astype(BF), du.astype(BF)
            act3[tok, cd] = ab
            act3[tok, cg] = dgb
            act3[tok, cu] = dub
            acc_o[...] += _nn(ab, w3[cd, :])
            dl = _nn(dgb, w3[cg, :]) + _nn(dub, w3[cu, :])
            if n == 0:
                acc_d[...] = dl
            else:
                acc_d[...] += dl
            if n == 1:
                zero_acc(i * TB + W)
            if n == 2:
                go_t[:, tok] = gb.astype(F32).T.astype(BF)

        out_st[...] = acc_o[...].astype(BF)
        list(nxt)
        dh = gb.astype(F32) + _ln_bwd(acc_d[...], h_v[...], rstd2)
        dh_v[tok, :] = dh
        do_t[...] = _nt(dh.astype(BF), wqo[:, 3 * D:]).T * linv[...]

        out_copy(i).start()
        pl.when(i < NB - 1)(lambda: attention(i, True, True))
        pl.when(i == NB - 1)(lambda: attention(i, True, False))
        return c

    lax.fori_loop(0, NB, block, 0)
    out_copy(NB - 1).wait()

    dx_copy = lambda i: pltpu.make_async_copy(
        go_v.at[_ds(i * TB, TB, TB), :], dx_h.at[_ds(i * TB, TB, TB), :], osem.at[1])

    def fin(i):
        tok = _ds(i * TB, TB, TB)
        ptok = _ds(i * TB + W, TB, TB)
        pm = _ds(i * TB + W - 128, 128, 128)
        dqb = (dq_t[:, tok] * 0.25).astype(BF)

        def gather(ra, rb):
            full = [ra[p][:, ptok] + jnp.concatenate(
                [rb[p][:, pm][:, 64:], rb[p][:, ptok][:, :TB - 64]], axis=1) for p in range(4)]
            return jnp.concatenate(
                [full[p][g * 32:g * 32 + 32] for g in range(4) for p in range(4)], axis=0)
        dkb16 = (gather(dka, dkb) * (1.0 / LOG2E)).astype(BF)
        dvb16 = gather(dva, dvb).astype(BF)
        dqkv_t[0:D, tok] = dqb
        dqkv_t[D:2 * D, tok] = dkb16
        dqkv_t[2 * D:3 * D, tok] = dvb16
        dqkv_t[3 * D:, tok] = dh_v[tok, :].T.astype(BF)
        dl = (_nn(wqo[:, 0:D], dqb) + _nn(wqo[:, D:2 * D], dkb16)
              + _nn(wqo[:, 2 * D:3 * D], dvb16))
        for p in range(4):
            dva[p][:, ptok] = dl[p * 128:(p + 1) * 128]

    def fin2(i):
        tok = _ds(i * TB, TB, TB)
        ptok = _ds(i * TB + W, TB, TB)
        dl = jnp.concatenate([dva[p][:, ptok].T for p in range(4)], axis=1)
        xh, rstd = _ln(x_v[tok, :].astype(F32))
        go_v[tok, :] = (dh_v[tok, :] + _ln_bwd(dl, xh, rstd)).astype(BF)

    cp_wg = pltpu.make_async_copy(wg, dwg_h, osem.at[2])
    cp_wu = pltpu.make_async_copy(wu, dwu_h, osem.at[3])
    cp_wd = pltpu.make_async_copy(wd, dwd_h, osem.at[4])
    cp_wq = pltpu.make_async_copy(wqkv, dwqkv_h, osem.at[5])
    cp_wo = [pltpu.make_async_copy(wqo.at[:, 3 * D + c:3 * D + c + 256], dwo_h.at[:, c:c + 256],
                                   osem.at[6 + c // 256]) for c in (0, 256)]

    cp_wg.start()

    @pl.loop(0, NB)
    def _(i):
        mlp_dw(i + NIT)
        fin(i)
        pl.when(i == 2)(lambda: cp_wu.start())

    w3[4096:, :] = _nn(lhs2[1], act3[:, 4096:]).T.astype(BF)
    now(lambda: cp_wd.start())

    @pl.loop(0, NB)
    def _(j):
        c = _ds(j * 256, 256, 256)
        wqo[:, c] = _nt(lhs1[j // 6], dqkv_t[c, :]).astype(BF)
        fin2(j)
        dx_copy(j).start()
        pl.when(j == 5)(lambda: cp_wq.start())
        pl.when(j == 6)(lambda: cp_wo[0].start())

    cp_wo[1].start()
    for i in range(NB):
        dx_copy(i).wait()
    for cp in (cp_wg, cp_wu, cp_wd, cp_wq, *cp_wo):
        cp.wait()


@jax.jit
def pallas_sequential_preLN__sliding_block__glu_gated_glu__prompt_kernel(
    A_x, A_wqkv, A_wo, B_x, B_w_gate, B_w_up, B_w_down, grad_out,
):
    V = pltpu.VMEM
    SP = S + W
    scratch = [
        V((S, D), BF), V((S, D), BF), V((D, 4 * D), BF),
        V((3 * FP, D), BF),
        V((SP // 2, D), jnp.int32), V((SP // 2, D), jnp.int32),
        V((D, SP), BF), V((D, SP), BF), V((D, SP), BF), V((D, SP), BF),
        V((D, S), BF), V((D, S), F32),
        *[[V((D // 4, SP), F32)] * 4] * 4,
        [V((2 * NSUB * 4, 320, 128), jnp.int32)] * 4, V((D, TB), F32),
        V((S, 3 * FP), BF), V((2, D, S), BF), V((2, D, S), BF),
        V((D, TB), F32), V((S, D), F32),
        V((TB, D), F32), V((TB, D), F32), V((TB, D), F32),
        V((TB, D), BF), V((4 * D, S), BF), [V((256, 512), F32)] * 2, [V((8, 512), F32)] * 2, V((4, 320, 128), jnp.int32), V((4, TB, 128), F32),
        pltpu.SemaphoreType.DMA((12,)), pltpu.SemaphoreType.DMA((8,)),
    ]
    sd = jax.ShapeDtypeStruct
    outs = pl.pallas_call(
        _kernel,
        grid=(1,),
        out_shape=(sd((S, D), BF), sd((S, D), BF), sd((D, 3 * D), BF), sd((D, D), BF),
                   sd((F, D), BF), sd((F, D), BF), sd((F, D), BF)),
        in_specs=[pl.BlockSpec(memory_space=pl.ANY)] * 7,
        out_specs=[pl.BlockSpec(memory_space=pl.ANY)] * 7,
        scratch_shapes=scratch,
        compiler_params=pltpu.CompilerParams(vmem_limit_bytes=126 * 1024 * 1024),
    )(A_x.reshape(S, D), A_wqkv, A_wo, B_w_gate.T, B_w_up.T, B_w_down, grad_out.reshape(S, D))
    return (outs[0].reshape(1, S, D), outs[1].reshape(1, S, D)) + (
        outs[2], outs[3], outs[4].T, outs[5].T, outs[6])
```
